```python
import os as _os
_os.environ.setdefault("JAX_PLATFORMS", "cpu")
import jax
import jax.numpy as jnp

def _softmax(x, axis=-1):
    return jax.nn.softmax(x, axis=axis)
def _gelu(x):
    return jax.nn.gelu(x, approximate=True)
def _silu(x):
    return jax.nn.silu(x)
def _sigmoid(x):
    return jax.nn.sigmoid(x)
def _layernorm(x, axis=-1, eps=1e-5):
    m = jnp.mean(x, axis=axis, keepdims=True)
    v = jnp.var(x, axis=axis, keepdims=True)
    return (x - m) / jnp.sqrt(v + eps)
def _scatter_add(tgt, idx, src, axis=0):
    return tgt.at[idx].add(src)
def _segment_sum(src, seg, n):
    return jax.ops.segment_sum(src, seg, n)
class _Rng:
    def __init__(self, key):
        self._k = key
    def _next(self):
        self._k, sub = jax.random.split(self._k)
        return sub
    def normal(self, shape):
        return jax.random.normal(self._next(), shape, dtype=jnp.bfloat16)
    def randint(self, lo, hi, shape):
        return jax.random.randint(self._next(), shape, lo, hi, dtype=jnp.int32)
    def uniform(self, shape, lo=0.0, hi=1.0):
        return jax.random.uniform(self._next(), shape, jnp.bfloat16, lo, hi)
    def permutation(self, n):
        return jax.random.permutation(self._next(), n)


kernel_name = 'gated_mix__linear_attn_block__sliding_local_dilated__prompt'

def setup_inputs():
    _rng = _Rng(jax.random.key(int.from_bytes(__import__("os").urandom(4), "little")))
    _w = (lambda a: (lambda t: t.astype(jnp.bfloat16) if jnp.issubdtype(t.dtype, jnp.floating) else t)(jnp.asarray(a)))
    def _A_setup():
        B, S, D = 1, 2048, 512
        return {
            "x": _w((lambda *s: _rng.normal(s) * 0.05)(B, S, D)),
            "wqkv": _w((lambda *s: _rng.normal(s) * 1.6)(D, 3 * D)),
            "wo": _w((lambda *s: _rng.normal(s) * 0.8)(D, D)),
        }
    _A_in = _A_setup()

    def _B_setup():
        B, S, D = 1, 2048, 512
        return {
            "x": _w((lambda *s: _rng.normal(s) * 0.05)(B, S, D)),
            "wqkv": _w((lambda *s: _rng.normal(s) * 0.8)(D, 3 * D)),
            "wo": _w((lambda *s: _rng.normal(s) * 0.05)(D, D)),
        }
    _B_in = _B_setup()

    return {
        "A_x": _A_in["x"],
        "A_wqkv": _A_in["wqkv"],
        "A_wo": _A_in["wo"],
        "B_x": _B_in["x"],
        "B_wqkv": _B_in["wqkv"],
        "B_wo": _B_in["wo"],
        "gate_w": _w((lambda *s: _rng.normal(s) * 0.05)(512) * 16.0),
    }

def reference(A_x, A_wqkv, A_wo, B_x, B_wqkv, B_wo, gate_w):
    def _A_ref(x, wqkv, wo):
        B, S, D = x.shape
        H = 32; Dh = D // H
        qkv = (lambda x, *d: x.transpose(*d))((x @ wqkv).reshape(B, S, 3, H, Dh), 2, 0, 3, 1, 4)
        q, k, v = qkv[0], qkv[1], qkv[2]
        phi = lambda t: jnp.where(t > 0, t + 1, jnp.exp(t)) + 1e-6
        pq, pk = phi(q), phi(k)
        kv = jnp.einsum("bhsd,bhse->bhde", pk, v)
        z = jnp.einsum("bhsd->bhd", pk)
        num = jnp.einsum("bhqd,bhde->bhqe", pq, kv)
        den = jnp.einsum("bhqd,bhd->bhq", pq, z)[..., None] + 1e-6
        o = num / den
        return (lambda x, *d: x.transpose(*d))(o, 0, 2, 1, 3).reshape(B, S, D) @ wo

    def _B_ref(x, wqkv, wo):
        B, S, D = x.shape
        H = 32; Dh = D // H
        W, dil = 8, 2
        qkv = (lambda x, *d: x.transpose(*d))((x @ wqkv).reshape(B, S, 3, H, Dh), 2, 0, 3, 1, 4)
        q, k, v = qkv[0], qkv[1], qkv[2]
        scale = Dh ** -0.5
        pos = jnp.arange(S)
        off = jnp.arange(W) * dil
        idx = pos[:, None] - off[None, :]
        mask = idx >= 0
        idx_c = jnp.where(mask, idx, 0).reshape(-1)
        kg = k[:, :, idx_c, :].reshape(B, H, S, W, Dh)
        vg = v[:, :, idx_c, :].reshape(B, H, S, W, Dh)
        logits = jnp.einsum("bhsd,bhswd->bhsw", q, kg) * scale
        logits = jnp.where(mask[None, None, :, :], logits, -1e9)
        attn = _softmax(logits, axis=-1)
        o = jnp.einsum("bhsw,bhswd->bhsd", attn, vg)
        return (lambda x, *d: x.transpose(*d))(o, 0, 2, 1, 3).reshape(B, S, D) @ wo

    x = A_x
    g = _sigmoid((x * gate_w).sum(-1, keepdims=True))
    a = _A_ref(x, A_wqkv, A_wo)
    b = _B_ref(x, B_wqkv, B_wo)
    return g * a + (1 - g) * b
```

```python
import functools
import jax
import jax.numpy as jnp
from jax import lax
import jax.experimental.pallas as pl
import jax.experimental.pallas.tpu as pltpu

S, D, H, DH = 2048, 512, 32, 16
W, DIL = 8, 2
TS = 256
NT = S // TS
HALO = 16
PS = 17
F32 = jnp.float32
BF16 = jnp.bfloat16
LOG2E = 1.4426950408889634
NT_DIMS = (((1,), (1,)), ((), ()))
MODE_LONG = (8, False)
MODE_LAST = (8, False)
P1T = 1
NP1 = NT // P1T


def _phi(t):
    return jnp.where(t > 0, t + 1.0, jnp.exp(t)) + 1e-6


def _dot(a, b):
    return jnp.dot(a, b, preferred_element_type=F32)


def _dot_nt(a, b):
    return lax.dot_general(a, b, NT_DIMS, preferred_element_type=F32)


def _rcp(x):
    r = pl.reciprocal(x, approx=True)
    return r * (2.0 - x * r)


def _kernel(x_hbm, wa_hbm, woa_hbm, wb_hbm, wob_hbm, gw_hbm, o_hbm,
            x_ref, wk_ref, wnat_ref, wv_ref, woa_ref, wob_ref, gw_ref,
            wkT_ref, g_ref, z_ref, tmp_ref, w2T_ref, wout_ref, m_ref, zrow_ref,
            k_ref, v_ref, q_ref, lhs_ref, ob_ref,
            sem_x, sem_w, sem_m, sem_o, sem_b):
    def barrier():
        pl.semaphore_signal(sem_b, 1)
        pl.semaphore_wait(sem_b, 1)

    def cp_x(i):
        n = P1T * TS
        return pltpu.make_async_copy(x_hbm.at[pl.ds(i * n, n), :], x_ref.at[pl.ds(i * n, n), :], sem_x.at[i])

    def cp_w(i):
        if isinstance(i, int) and i < 2:
            src = wa_hbm.at[:, pl.ds(i * 256, 256)]
        elif isinstance(i, int):
            src = wb_hbm.at[:, pl.ds((i - 2) * 256, 256)]
        else:
            src = wb_hbm.at[:, pl.ds(pl.multiple_of((i - 2) * 256, 256), 256)]
        return pltpu.make_async_copy(src, wnat_ref.at[i], sem_w.at[i])

    def cp_w_wait(i):
        return pltpu.make_async_copy(wnat_ref.at[i], wnat_ref.at[i], sem_w.at[i])

    def cp_wk(hf):
        return pltpu.make_async_copy(wa_hbm.at[:, pl.ds(D + hf * 256, 256)], wk_ref.at[hf], sem_m.at[5 + hf])

    cp_wv = pltpu.make_async_copy(wa_hbm.at[:, pl.ds(2 * D, D)], wv_ref, sem_m.at[1])
    cp_woa = pltpu.make_async_copy(woa_hbm, woa_ref, sem_m.at[2])
    cp_wob = pltpu.make_async_copy(wob_hbm, wob_ref, sem_m.at[3])
    cp_gw = pltpu.make_async_copy(gw_hbm, gw_ref, sem_m.at[4])

    def cp_o(i):
        return pltpu.make_async_copy(ob_ref.at[pl.ds(i * TS, TS), :], o_hbm.at[pl.ds(i * TS, TS), :], sem_o.at[i])

    def prep_w(i, u):
        wt = wnat_ref[i].astype(F32).T
        for hh in range(16):
            for j in range(4):
                tmp_ref[u, j, PS * hh:PS * hh + DH, :] = wt[DH * hh:DH * (hh + 1), 128 * j:128 * (j + 1)]
        base = (i // 2) * D + (i % 2) * 16
        for d in range(DH):
            r = base + d * 32
            if not isinstance(r, int):
                r = pl.multiple_of(r, 16)
            for j in range(4):
                w2T_ref[pl.ds(r, 16), 128 * j:128 * (j + 1)] = tmp_ref[u, j, pl.ds(d, 16, stride=PS), :].astype(BF16)

    cp_x(0).start()
    cp_wk(0).start()
    cp_wk(1).start()
    k_ref[:, 0:HALO, :] = jnp.zeros((4, HALO, 128), F32)
    v_ref[:, 0:HALO, :] = jnp.zeros((4, HALO, 128), F32)

    for hf in range(2):
        if hf == 0:
            cp_x(0).wait()
        cp_wk(hf).wait()
        if hf == 0:
            cp_x(1).start()
            cp_w(0).start()
        else:
            cp_x(2).start()
            cp_w(1).start()
        x0 = x_ref[0:TS, :]
        pkT = _phi(_dot(x0, wk_ref[hf])).T
        zs = pkT[:, 0:128]
        for j in range(1, TS // 128):
            zs = zs + pkT[:, 128 * j:128 * (j + 1)]
        z_ref[hf * 256:(hf + 1) * 256, :] = zs
        g_ref[hf * 256:(hf + 1) * 256, :] = _dot(pkT.astype(BF16), x0)
        wkT_ref[hf * 256:(hf + 1) * 256, :] = wk_ref[hf].astype(F32).T.astype(BF16)

    def p1(it, carry):
        @pl.when(it + 2 < NP1)
        def _():
            cp_x(it + 2).start()

        @pl.when(it + 1 < NP1)
        def _():
            cp_w(it + 1).start()

        @pl.when(it == NP1 - 2)
        def _():
            cp_wv.start()
            cp_woa.start()
            cp_wob.start()
            cp_gw.start()

        cp_x(it).wait()
        cp_w_wait(it - 1).wait()
        n = TS
        r0 = pl.multiple_of(it * n, n)
        xt = x_ref[pl.ds(r0, n), :]
        kT = _dot_nt(wkT_ref[...], xt)
        pk = _phi(kT)
        zs = pk[:, 0:128]
        for j in range(1, n // 128):
            zs = zs + pk[:, 128 * j:128 * (j + 1)]
        z_ref[...] += zs
        g_ref[...] += _dot(pk.astype(BF16), xt)
        prep_w(it - 1, 0)
        return carry

    lax.fori_loop(1, NP1, p1, 0)

    def proj(i, part):
        r0 = i * TS
        xt = x_ref[r0:r0 + TS, :]
        pr = _dot_nt(xt, w2T_ref[part * D:(part + 1) * D, :])
        if part == 0:
            q_ref[r0:r0 + TS, 0:D] = pr
        elif part == 1:
            q_ref[r0:r0 + TS, D:2 * D] = pr * (0.25 * LOG2E)
        else:
            dst = k_ref if part == 2 else v_ref
            for j in range(4):
                dst[j, HALO + r0:HALO + r0 + TS, :] = pr[:, 128 * j:128 * (j + 1)]

    def attn(i, mode):
        CH, pipelined = mode
        r0 = i * TS
        zrow = zrow_ref[0:1, :]
        gw = gw_ref[...].reshape(1, D).astype(F32)
        nch = TS // CH

        def stage1(c):
            a0 = r0 + c * CH
            gs = jnp.sum(x_ref[a0:a0 + CH, :].astype(F32) * gw, axis=1, keepdims=True)
            pq = _phi(q_ref[a0:a0 + CH, 0:D])
            t = pq * zrow
            t = t[:, 0:128] + t[:, 128:256] + t[:, 256:384] + t[:, 384:512]
            q = [q_ref[a0:a0 + CH, D + 128 * j:D + 128 * (j + 1)] for j in range(4)]
            ls = [t]
            for w in range(W):
                st = HALO + a0 - DIL * w
                l = q[0] * k_ref[0, st:st + CH, :]
                for j in range(1, 4):
                    l = l + q[j] * k_ref[j, st:st + CH, :]
                ls.append(l)
            rs = [pltpu.roll(l, 64, 1) for l in ls]
            return gs, pq, ls, rs

        def stage2(st1):
            gs, pq, ls, rs = st1
            ls = [l + r for l, r in zip(ls, rs)]
            rs = [pltpu.roll(l, 32, 1) for l in ls]
            return gs, pq, ls, rs

        def stage3(c, st2):
            a0 = r0 + c * CH
            gs, pq, ls, rs = st2
            ls = [l + r for l, r in zip(ls, rs)]
            g = jax.nn.sigmoid(gs)
            fa = g * _rcp(ls[0] + 1e-6)
            ls = ls[1:]
            if a0 < HALO:
                row = a0 + lax.broadcasted_iota(jnp.int32, (CH, 128), 0)
                ls = [ls[0]] + [jnp.where(row >= DIL * w, ls[w], -1e9 * LOG2E) for w in range(1, W)]
            m = ls[0]
            for w in range(1, W):
                m = jnp.maximum(m, ls[w])
            es = [jnp.exp2(l - m) for l in ls]
            den = es[0]
            for w in range(1, W):
                den = den + es[w]
            fb = (1.0 - g) * _rcp(den)
            for j in range(4):
                acc = None
                for w in range(W):
                    st = HALO + a0 - DIL * w
                    term = es[w] * v_ref[j, st:st + CH, :]
                    acc = term if acc is None else acc + term
                lhs_ref[a0:a0 + CH, D + 128 * j:D + 128 * (j + 1)] = (acc * fb).astype(BF16)
                lhs_ref[a0:a0 + CH, 128 * j:128 * (j + 1)] = (pq[:, 128 * j:128 * (j + 1)] * fa).astype(BF16)

        if pipelined:
            s1 = {}
            s2 = {}
            for c in range(nch + 2):
                if c < nch:
                    s1[c] = stage1(c)
                if 0 <= c - 1 < nch:
                    s2[c - 1] = stage2(s1.pop(c - 1))
                if 0 <= c - 2 < nch:
                    stage3(c - 2, s2.pop(c - 2))
        else:
            for c in range(nch):
                stage3(c, stage2(stage1(c)))

    def outp(i, half):
        r0 = i * TS
        c0 = half * 256
        ob_ref[r0:r0 + TS, c0:c0 + 256] = _dot(lhs_ref[r0:r0 + TS, :], wout_ref[:, c0:c0 + 256]).astype(BF16)

    def perm_rows_store(slot, val, c):
        for hh in range(8):
            p0 = PS * (8 * c + hh)
            for j in range(val.shape[1] // 128):
                m_ref[slot + j, p0:p0 + DH, :] = val[DH * hh:DH * (hh + 1), 128 * j:128 * (j + 1)]

    def perm_rows_load(slot, row0):
        for d in range(DH):
            for j in range(4):
                wout_ref[row0 + d * 32:row0 + (d + 1) * 32, 128 * j:128 * (j + 1)] = (
                    m_ref[slot + j, pl.ds(d, 32, stride=PS), :].astype(BF16))

    cp_wv.wait()
    cp_woa.wait()
    cp_wob.wait()
    cp_gw.wait()
    cp_w(NT - 1).wait()
    prep_w(NT - 1, 0)
    for c in range(4):
        perm_rows_store(8, z_ref[128 * c:128 * (c + 1), :], c)
    zp = jnp.concatenate([m_ref[8, pl.ds(d, 32, stride=PS), :] for d in range(DH)], axis=0)
    zrow_ref[...] = jnp.broadcast_to(jnp.sum(zp.T, axis=0, keepdims=True), (8, D))
    r_i = lax.broadcasted_iota(jnp.int32, (128, 128), 0) // DH
    c_i = lax.broadcasted_iota(jnp.int32, (128, 128), 1) // DH
    bd = r_i == c_i
    kvs = []
    for c in range(4):
        gc = g_ref[128 * c:128 * (c + 1), :].astype(BF16)
        kvs.append(jnp.where(bd, _dot(gc, wv_ref[:, 128 * c:128 * (c + 1)]), 0.0).astype(BF16))
    proj(0, 0)
    for c in range(4):
        mc = _dot(kvs[c], woa_ref[128 * c:128 * (c + 1), :])
        perm_rows_store(0, mc, c)
    proj(0, 1)
    proj(0, 2)
    proj(0, 3)

    P = lambda i: [("P", i, p) for p in range(4)]
    O = lambda t: [("O", t, 0), ("O", t, 1)]
    sched = [
        P(1) + P(2)[:1],
        P(2)[1:] + O(0),
        P(3) + O(1)[:1],
        P(4) + O(1)[1:],
        P(5) + O(2)[:1],
        P(6) + O(2)[1:],
        P(7) + O(3),
        O(4) + O(5) + O(6),
    ]
    pending = []
    for i in range(NT):
        barrier()
        for t in pending:
            cp_o(t).start()
        pending = []
        if i == 0:
            perm_rows_load(0, 0)
            for c in range(4):
                perm_rows_store(4, wob_ref[128 * c:128 * (c + 1), :].astype(F32), c)
            perm_rows_load(4, D)
        for (kind, t, p) in sched[i]:
            if kind == "P":
                proj(t, p)
            else:
                outp(t, p)
                if p == 1:
                    pending.append(t)
        attn(i, MODE_LAST if i == NT - 1 else MODE_LONG)
    barrier()
    for t in pending:
        cp_o(t).start()
    outp(NT - 1, 0)
    outp(NT - 1, 1)
    cp_o(NT - 1).start()
    for t in range(NT):
        cp_o(t).wait()


@jax.jit
def pallas_gated_mix__linear_attn_block__sliding_local_dilated__prompt_kernel(
    A_x, A_wqkv, A_wo, B_x, B_wqkv, B_wo, gate_w,
):
    x = A_x.reshape(S, D)
    any_spec = pl.BlockSpec(memory_space=pl.ANY)
    out = pl.pallas_call(
        _kernel,
        out_shape=jax.ShapeDtypeStruct((S, D), BF16),
        in_specs=[any_spec] * 6,
        out_specs=any_spec,
        scratch_shapes=[
            pltpu.VMEM((S, D), BF16),
            pltpu.VMEM((2, D, 256), BF16),
            pltpu.VMEM((NT, D, 256), BF16),
            pltpu.VMEM((D, D), BF16),
            pltpu.VMEM((D, D), BF16),
            pltpu.VMEM((D, D), BF16),
            pltpu.VMEM((D,), BF16),
            pltpu.VMEM((D, D), BF16),
            pltpu.VMEM((D, D), F32),
            pltpu.VMEM((D, 128), F32),
            pltpu.VMEM((P1T, 4, 16 * PS, 128), F32),
            pltpu.VMEM((4 * D, D), BF16),
            pltpu.VMEM((2 * D, D), BF16),
            pltpu.VMEM((9, 32 * PS, 128), F32),
            pltpu.VMEM((8, D), F32),
            pltpu.VMEM((4, HALO + S, 128), F32),
            pltpu.VMEM((4, HALO + S, 128), F32),
            pltpu.VMEM((S, 2 * D), F32),
            pltpu.VMEM((S, 2 * D), BF16),
            pltpu.VMEM((S, D), BF16),
            pltpu.SemaphoreType.DMA((NP1,)),
            pltpu.SemaphoreType.DMA((NT,)),
            pltpu.SemaphoreType.DMA((7,)),
            pltpu.SemaphoreType.DMA((NT,)),
            pltpu.SemaphoreType.REGULAR,
        ],
        compiler_params=pltpu.CompilerParams(vmem_limit_bytes=100 * 1024 * 1024),
    )(x, A_wqkv, A_wo, B_wqkv, B_wo, gate_w)
    return out.reshape(1, S, D)
```

```python
import jax
import jax.numpy as jnp
from jax import lax
import jax.experimental.pallas as pl
import jax.experimental.pallas.tpu as pltpu

S, D, H, DH = 2048, 512, 32, 16
W, DIL = 8, 2
TS = 256
NT = S // TS
HALO = 16
PS = 17
F32 = jnp.float32
BF16 = jnp.bfloat16
LOG2E = 1.4426950408889634
NT_DIMS = (((1,), (1,)), ((), ()))
NFS = [4, 4, 4, 4]


def _phi(t):
    return jnp.where(t > 0, t + 1.0, jnp.exp(t)) + 1e-6


def _dot(a, b):
    return jnp.dot(a, b, preferred_element_type=F32)


def _dot_nt(a, b):
    return lax.dot_general(a, b, NT_DIMS, preferred_element_type=F32)


def _rcp(x):
    r = pl.reciprocal(x, approx=True)
    return r * (2.0 - x * r)


def _kernel(x_hbm, wa_hbm, woa_hbm, wb_hbm, wob_hbm, gw_hbm, o_hbm,
            x_ref, wk_ref, wnat_ref, wv_ref, woa_ref, wob_ref, gw_ref,
            wkT_ref, g_ref, z_ref, tmp_ref, w2T_ref, wout_ref, m_ref, zrow_ref,
            k_ref, v_ref, q_ref, lhs_ref, ob_ref,
            sem_x, sem_w, sem_m, sem_o, sem_b):
    def barrier():
        pl.semaphore_signal(sem_b, 1)
        pl.semaphore_wait(sem_b, 1)

    def cp_x1(i):
        return pltpu.make_async_copy(x_hbm.at[pl.ds(i * TS, TS), :], x_ref.at[pl.ds(i * TS, TS), :], sem_m.at[7 + i])

    def cp_x2(p):
        r = p * 2 * TS
        if not isinstance(p, int):
            r = pl.multiple_of(r, 2 * TS)
        return pltpu.make_async_copy(x_hbm.at[pl.ds(r, 2 * TS), :], x_ref.at[pl.ds(r, 2 * TS), :], sem_x.at[p])

    def cp_w(m):
        src = wa_hbm.at[:, pl.ds(0, D)] if m == 0 else wb_hbm.at[:, pl.ds((m - 1) * D, D)]
        return pltpu.make_async_copy(src, wnat_ref.at[m], sem_w.at[m])

    def cp_w_wait(m):
        return pltpu.make_async_copy(wnat_ref.at[m], wnat_ref.at[m], sem_w.at[m])

    def cp_wk(hf):
        return pltpu.make_async_copy(wa_hbm.at[:, pl.ds(D + hf * 256, 256)], wk_ref.at[hf], sem_m.at[5 + hf])

    cp_wv = pltpu.make_async_copy(wa_hbm.at[:, pl.ds(2 * D, D)], wv_ref, sem_m.at[1])
    cp_woa = pltpu.make_async_copy(woa_hbm, woa_ref, sem_m.at[2])
    cp_wob = pltpu.make_async_copy(wob_hbm, wob_ref, sem_m.at[3])
    cp_gw = pltpu.make_async_copy(gw_hbm, gw_ref, sem_m.at[4])

    def cp_o(i):
        return pltpu.make_async_copy(ob_ref.at[pl.ds(i * TS, TS), :], o_hbm.at[pl.ds(i * TS, TS), :], sem_o.at[i])

    def prep_w(m):
        for hf in range(2):
            wt = wnat_ref[m, :, hf * 256:(hf + 1) * 256].astype(F32).T
            for hh in range(16):
                for j in range(4):
                    tmp_ref[2 * m + hf, j, PS * hh:PS * hh + DH, :] = wt[DH * hh:DH * (hh + 1), 128 * j:128 * (j + 1)]
            base = m * D + hf * 16
            for d in range(DH):
                r = base + d * 32
                if not isinstance(r, int):
                    r = pl.multiple_of(r, 16)
                for j in range(4):
                    w2T_ref[pl.ds(r, 16), 128 * j:128 * (j + 1)] = tmp_ref[2 * m + hf, j, pl.ds(d, 16, stride=PS), :].astype(BF16)

    cp_x1(0).start()
    cp_wk(0).start()
    cp_wk(1).start()
    cp_x1(1).start()
    cp_x2(1).start()
    cp_x2(2).start()
    k_ref[:, 0:HALO, :] = jnp.zeros((4, HALO, 128), F32)
    v_ref[:, 0:HALO, :] = jnp.zeros((4, HALO, 128), F32)

    for hf in range(2):
        cp_x1(hf).wait()
        cp_wk(hf).wait()
        if hf == 0:
            cp_x2(3).start()
            cp_w(0).start()
            cp_w(1).start()
            cp_w(2).start()
        else:
            cp_w(3).start()
            cp_wv.start()
            cp_woa.start()
            cp_wob.start()
            cp_gw.start()
        x0 = x_ref[0:TS, :]
        pkT = _phi(_dot(x0, wk_ref[hf])).T
        zs = pkT[:, 0:128]
        for j in range(1, TS // 128):
            zs = zs + pkT[:, 128 * j:128 * (j + 1)]
        z_ref[hf * 256:(hf + 1) * 256, :] = zs
        g_ref[hf * 256:(hf + 1) * 256, :] = _dot(pkT.astype(BF16), x0)
        wkT_ref[hf * 256:(hf + 1) * 256, :] = wk_ref[hf].astype(F32).T.astype(BF16)

    def p1_seg(t0, nt):
        n = nt * TS
        r0 = t0 * TS if isinstance(t0, int) else pl.multiple_of(t0 * TS, TS)
        xt = x_ref[pl.ds(r0, n), :]
        kT = _dot_nt(wkT_ref[...], xt)
        pk = _phi(kT)
        zs = pk[:, 0:128]
        for j in range(1, n // 128):
            zs = zs + pk[:, 128 * j:128 * (j + 1)]
        z_ref[...] += zs
        g_ref[...] += _dot(pk.astype(BF16), xt)

    p1_seg(1, 1)

    cp_x2(1).wait()
    cp_x2(2).wait()
    p1_seg(2, 2)
    p1_seg(4, 2)

    def proj(i, part):
        r0 = i * TS
        xt = x_ref[r0:r0 + TS, :]
        pr = _dot_nt(xt, w2T_ref[part * D:(part + 1) * D, :])
        if part == 0:
            q_ref[r0:r0 + TS, 0:D] = pr
        elif part == 1:
            q_ref[r0:r0 + TS, D:2 * D] = pr * (0.25 * LOG2E)
        else:
            dst = k_ref if part == 2 else v_ref
            for j in range(4):
                dst[j, HALO + r0:HALO + r0 + TS, :] = pr[:, 128 * j:128 * (j + 1)]

    def attn(i, pattern):
        r0 = i * TS
        zrow = zrow_ref[0:1, :]
        gw = gw_ref[...].reshape(1, D).astype(F32)

        def stage1(a0, CH):
            gs = jnp.sum(x_ref[a0:a0 + CH, :].astype(F32) * gw, axis=1, keepdims=True)
            pq = _phi(q_ref[a0:a0 + CH, 0:D])
            t = pq * zrow
            t = t[:, 0:128] + t[:, 128:256] + t[:, 256:384] + t[:, 384:512]
            q = [q_ref[a0:a0 + CH, D + 128 * j:D + 128 * (j + 1)] for j in range(4)]
            ls = [t]
            for w in range(W):
                st = HALO + a0 - DIL * w
                l = q[0] * k_ref[0, st:st + CH, :]
                for j in range(1, 4):
                    l = l + q[j] * k_ref[j, st:st + CH, :]
                ls.append(l)
            rs = [pltpu.roll(l, 64, 1) for l in ls]
            return gs, pq, ls, rs

        def stage2(st1):
            gs, pq, ls, rs = st1
            ls = [l + r for l, r in zip(ls, rs)]
            rs = [pltpu.roll(l, 32, 1) for l in ls]
            return gs, pq, ls, rs

        def stage3(a0, CH, st2):
            gs, pq, ls, rs = st2
            ls = [l + r for l, r in zip(ls, rs)]
            g = jax.nn.sigmoid(gs)
            fa = g * _rcp(ls[0] + 1e-6)
            ls = ls[1:]
            if a0 < HALO:
                row = a0 + lax.broadcasted_iota(jnp.int32, (CH, 128), 0)
                ls = [ls[0]] + [jnp.where(row >= DIL * w, ls[w], -1e9 * LOG2E) for w in range(1, W)]
            m = ls[0]
            for w in range(1, W):
                m = jnp.maximum(m, ls[w])
            es = [jnp.exp2(l - m) for l in ls]
            den = es[0]
            for w in range(1, W):
                den = den + es[w]
            fb = (1.0 - g) * _rcp(den)
            for j in range(4):
                acc = None
                for w in range(W):
                    st = HALO + a0 - DIL * w
                    term = es[w] * v_ref[j, st:st + CH, :]
                    acc = term if acc is None else acc + term
                lhs_ref[a0:a0 + CH, D + 128 * j:D + 128 * (j + 1)] = (acc * fb).astype(BF16)
                lhs_ref[a0:a0 + CH, 128 * j:128 * (j + 1)] = (pq[:, 128 * j:128 * (j + 1)] * fa).astype(BF16)

        a0 = r0
        for CH in pattern:
            stage3(a0, CH, stage2(stage1(a0, CH)))
            a0 += CH
        assert a0 == r0 + TS

    def outp(i, half):
        r0 = i * TS
        c0 = half * 256
        ob_ref[r0:r0 + TS, c0:c0 + 256] = _dot(lhs_ref[r0:r0 + TS, :], wout_ref[:, c0:c0 + 256]).astype(BF16)

    def perm_rows_store(slot, val, c):
        for hh in range(8):
            p0 = PS * (8 * c + hh)
            for j in range(val.shape[1] // 128):
                m_ref[slot + j, p0:p0 + DH, :] = val[DH * hh:DH * (hh + 1), 128 * j:128 * (j + 1)]

    def perm_rows_load(slot, row0):
        for d in range(DH):
            for j in range(4):
                wout_ref[row0 + d * 32:row0 + (d + 1) * 32, 128 * j:128 * (j + 1)] = (
                    m_ref[slot + j, pl.ds(d, 32, stride=PS), :].astype(BF16))

    for m in range(4):
        cp_w(m).wait()
    cp_wv.wait()
    cp_woa.wait()
    cp_wob.wait()
    cp_gw.wait()
    cp_x2(3).wait()
    p1_seg(6, 2)
    prep_w(0)
    for c in range(4):
        perm_rows_store(8, z_ref[128 * c:128 * (c + 1), :], c)
    zp = jnp.concatenate([m_ref[8, pl.ds(d, 32, stride=PS), :] for d in range(DH)], axis=0)
    zrow_ref[...] = jnp.broadcast_to(jnp.sum(zp.T, axis=0, keepdims=True), (8, D))
    r_i = lax.broadcasted_iota(jnp.int32, (128, 128), 0) // DH
    c_i = lax.broadcasted_iota(jnp.int32, (128, 128), 1) // DH
    bd = r_i == c_i
    kvs = []
    for c in range(4):
        gc = g_ref[128 * c:128 * (c + 1), :].astype(BF16)
        kvs.append(jnp.where(bd, _dot(gc, wv_ref[:, 128 * c:128 * (c + 1)]), 0.0).astype(BF16))
    for c in range(4):
        mc = _dot(kvs[c], woa_ref[128 * c:128 * (c + 1), :])
        perm_rows_store(0, mc, c)
    for p in range(4):
        if p > 0:
            prep_w(p)
        proj(0, p)
        proj(1, p)

    P = lambda i: [("P", i, p) for p in range(4)]
    O = lambda t: [("O", t, 0), ("O", t, 1)]
    sched = [
        P(2) + P(3) + P(4)[:1],
        P(4)[1:] + P(5) + O(0),
        P(6) + P(7) + O(1)[:1],
        O(1)[1:] + O(2) + O(3) + O(4) + O(5),
    ]

    def mk_pattern(nf):
        n8 = (TS - 16 * nf) // 8
        pattern = []
        for c in range(n8 + nf):
            if nf and (c * nf) // (n8 + nf) != ((c + 1) * nf) // (n8 + nf):
                pattern.append(16)
            else:
                pattern.append(8)
        return pattern

    pending = []
    for s in range(4):
        barrier()
        for t in pending:
            cp_o(t).start()
        pending = []
        if s == 0:
            perm_rows_load(0, 0)
            for c in range(4):
                perm_rows_store(4, wob_ref[128 * c:128 * (c + 1), :].astype(F32), c)
            perm_rows_load(4, D)
        for (kind, t, p) in sched[s]:
            if kind == "P":
                proj(t, p)
            else:
                outp(t, p)
                if p == 1:
                    if s == 3:
                        cp_o(t).start()
                    else:
                        pending.append(t)
        attn(2 * s, mk_pattern(NFS[s]))
        attn(2 * s + 1, mk_pattern(NFS[s]))
    barrier()
    outp(NT - 2, 0)
    outp(NT - 2, 1)
    cp_o(NT - 2).start()
    last = []
    r7 = (NT - 1) * TS
    for qt, (c0, nc) in enumerate([(0, 256), (256, 128), (384, 128)]):
        ob_ref[r7:r7 + TS, c0:c0 + nc] = _dot(lhs_ref[r7:r7 + TS, :], wout_ref[:, c0:c0 + nc]).astype(BF16)
        c = pltpu.make_async_copy(ob_ref.at[pl.ds(r7, TS), pl.ds(c0, nc)],
                                  o_hbm.at[pl.ds(r7, TS), pl.ds(c0, nc)], sem_o.at[NT - 1 + qt])
        c.start()
        last.append(c)
    for t in range(NT - 1):
        cp_o(t).wait()
    for c in last:
        c.wait()


@jax.jit
def pallas_gated_mix__linear_attn_block__sliding_local_dilated__prompt_kernel(
    A_x, A_wqkv, A_wo, B_x, B_wqkv, B_wo, gate_w,
):
    x = A_x.reshape(S, D)
    any_spec = pl.BlockSpec(memory_space=pl.ANY)
    out = pl.pallas_call(
        _kernel,
        out_shape=jax.ShapeDtypeStruct((S, D), BF16),
        in_specs=[any_spec] * 6,
        out_specs=any_spec,
        scratch_shapes=[
            pltpu.VMEM((S, D), BF16),
            pltpu.VMEM((2, D, 256), BF16),
            pltpu.VMEM((4, D, D), BF16),
            pltpu.VMEM((D, D), BF16),
            pltpu.VMEM((D, D), BF16),
            pltpu.VMEM((D, D), BF16),
            pltpu.VMEM((D,), BF16),
            pltpu.VMEM((D, D), BF16),
            pltpu.VMEM((D, D), F32),
            pltpu.VMEM((D, 128), F32),
            pltpu.VMEM((8, 4, 16 * PS, 128), F32),
            pltpu.VMEM((4 * D, D), BF16),
            pltpu.VMEM((2 * D, D), BF16),
            pltpu.VMEM((9, 32 * PS, 128), F32),
            pltpu.VMEM((8, D), F32),
            pltpu.VMEM((4, HALO + S, 128), F32),
            pltpu.VMEM((4, HALO + S, 128), F32),
            pltpu.VMEM((S, 2 * D), F32),
            pltpu.VMEM((S, 2 * D), BF16),
            pltpu.VMEM((S, D), BF16),
            pltpu.SemaphoreType.DMA((4,)),
            pltpu.SemaphoreType.DMA((4,)),
            pltpu.SemaphoreType.DMA((9,)),
            pltpu.SemaphoreType.DMA((NT + 2,)),
            pltpu.SemaphoreType.REGULAR,
        ],
        compiler_params=pltpu.CompilerParams(vmem_limit_bytes=100 * 1024 * 1024),
    )(x, A_wqkv, A_wo, B_wqkv, B_wo, gate_w)
    return out.reshape(1, S, D)
```

```python
import jax
import jax.numpy as jnp
from jax import lax
import jax.experimental.pallas as pl
import jax.experimental.pallas.tpu as pltpu

S, D, H, DH = 2048, 512, 32, 16
W, DIL = 8, 2
TS = 256
NT = S // TS
HALO = 16
PS = 17
F32 = jnp.float32
BF16 = jnp.bfloat16
LOG2E = 1.4426950408889634
NT_DIMS = (((1,), (1,)), ((), ()))
NFS = [4, 4, 4, 4]


def _phi(t):
    return jnp.where(t > 0, t + 1.0, jnp.exp(t)) + 1e-6


def _dot(a, b):
    return jnp.dot(a, b, preferred_element_type=F32)


def _dot_nt(a, b):
    return lax.dot_general(a, b, NT_DIMS, preferred_element_type=F32)


def _rcp(x):
    r = pl.reciprocal(x, approx=True)
    return r * (2.0 - x * r)


def _kernel(x_hbm, wa_hbm, woa_hbm, wb_hbm, wob_hbm, gw_hbm, o_hbm,
            x_ref, wk_ref, wnat_ref, wv_ref, woa_ref, wob_ref, gw_ref,
            wkT_ref, g_ref, z_ref, tmp_ref, w2T_ref, wout_ref, m_ref, zrow_ref,
            k_ref, v_ref, q_ref, lhs_ref, ob_ref,
            sem_d, sem_b):
    def barrier():
        pl.semaphore_signal(sem_b, 1)
        pl.semaphore_wait(sem_b, 1)

    def cp_x1(i):
        return pltpu.make_async_copy(x_hbm.at[pl.ds(i * TS, TS), :], x_ref.at[pl.ds(i * TS, TS), :], sem_d.at[i])

    def cp_x2(p):
        r = p * 2 * TS
        return pltpu.make_async_copy(x_hbm.at[pl.ds(r, 2 * TS), :], x_ref.at[pl.ds(r, 2 * TS), :],
                                     sem_d.at[2 if p < 3 else 3])

    def cp_w(m):
        src = wa_hbm.at[:, pl.ds(0, D)] if m == 0 else wb_hbm.at[:, pl.ds((m - 1) * D, D)]
        return pltpu.make_async_copy(src, wnat_ref.at[m], sem_d.at[3])

    def cp_wk(hf):
        return pltpu.make_async_copy(wa_hbm.at[:, pl.ds(D + hf * 256, 256)], wk_ref.at[hf], sem_d.at[hf])

    cp_wv = pltpu.make_async_copy(wa_hbm.at[:, pl.ds(2 * D, D)], wv_ref, sem_d.at[3])
    cp_woa = pltpu.make_async_copy(woa_hbm, woa_ref, sem_d.at[3])
    cp_wob = pltpu.make_async_copy(wob_hbm, wob_ref, sem_d.at[3])
    cp_gw = pltpu.make_async_copy(gw_hbm, gw_ref, sem_d.at[3])

    def cp_o(i):
        return pltpu.make_async_copy(ob_ref.at[pl.ds(i * TS, TS), :], o_hbm.at[pl.ds(i * TS, TS), :], sem_d.at[4])

    def prep_w(m):
        for hf in range(2):
            wt = wnat_ref[m, :, hf * 256:(hf + 1) * 256].astype(F32).T
            for hh in range(16):
                for j in range(4):
                    tmp_ref[2 * m + hf, j, PS * hh:PS * hh + DH, :] = wt[DH * hh:DH * (hh + 1), 128 * j:128 * (j + 1)]
            base = m * D + hf * 16
            for d in range(DH):
                r = base + d * 32
                for j in range(4):
                    w2T_ref[pl.ds(r, 16), 128 * j:128 * (j + 1)] = (
                        tmp_ref[2 * m + hf, j, pl.ds(d, 16, stride=PS), :].astype(BF16))

    cp_x1(0).start()
    cp_wk(0).start()
    cp_wk(1).start()
    cp_x1(1).start()
    cp_x2(1).start()
    cp_x2(2).start()
    k_ref[:, 0:HALO, :] = jnp.zeros((4, HALO, 128), F32)
    v_ref[:, 0:HALO, :] = jnp.zeros((4, HALO, 128), F32)

    for hf in range(2):
        cp_x1(hf).wait()
        cp_wk(hf).wait()
        if hf == 0:
            cp_x2(3).start()
            cp_w(0).start()
            cp_w(1).start()
            cp_w(2).start()
        else:
            cp_w(3).start()
            cp_wv.start()
            cp_woa.start()
            cp_wob.start()
            cp_gw.start()
        x0 = x_ref[0:TS, :]
        pkT = _phi(_dot(x0, wk_ref[hf])).T
        zs = pkT[:, 0:128]
        for j in range(1, TS // 128):
            zs = zs + pkT[:, 128 * j:128 * (j + 1)]
        z_ref[hf * 256:(hf + 1) * 256, :] = zs
        g_ref[hf * 256:(hf + 1) * 256, :] = _dot(pkT.astype(BF16), x0)
        wkT_ref[hf * 256:(hf + 1) * 256, :] = wk_ref[hf].astype(F32).T.astype(BF16)

    def p1_seg(t0, nt):
        n = nt * TS
        r0 = t0 * TS
        xt = x_ref[pl.ds(r0, n), :]
        kT = _dot_nt(wkT_ref[...], xt)
        pk = _phi(kT)
        zs = pk[:, 0:128]
        for j in range(1, n // 128):
            zs = zs + pk[:, 128 * j:128 * (j + 1)]
        z_ref[...] += zs
        g_ref[...] += _dot(pk.astype(BF16), xt)

    p1_seg(1, 1)

    cp_x2(1).wait()
    cp_x2(2).wait()
    p1_seg(2, 2)
    p1_seg(4, 2)

    def proj(i, part):
        r0 = i * TS
        xt = x_ref[r0:r0 + TS, :]
        pr = _dot_nt(xt, w2T_ref[part * D:(part + 1) * D, :])
        if part == 0:
            q_ref[r0:r0 + TS, 0:D] = pr
        elif part == 1:
            q_ref[r0:r0 + TS, D:2 * D] = pr * (0.25 * LOG2E)
        else:
            dst = k_ref if part == 2 else v_ref
            for j in range(4):
                dst[j, HALO + r0:HALO + r0 + TS, :] = pr[:, 128 * j:128 * (j + 1)]

    def attn(i, pattern):
        r0 = i * TS
        zrow = zrow_ref[0:1, :]
        gw = gw_ref[...].reshape(1, D).astype(F32)

        def stage1(a0, CH):
            gs = jnp.sum(x_ref[a0:a0 + CH, :].astype(F32) * gw, axis=1, keepdims=True)
            pq = _phi(q_ref[a0:a0 + CH, 0:D])
            t = pq * zrow
            t = t[:, 0:128] + t[:, 128:256] + t[:, 256:384] + t[:, 384:512]
            q = [q_ref[a0:a0 + CH, D + 128 * j:D + 128 * (j + 1)] for j in range(4)]
            ls = [t]
            for w in range(W):
                st = HALO + a0 - DIL * w
                l = q[0] * k_ref[0, st:st + CH, :]
                for j in range(1, 4):
                    l = l + q[j] * k_ref[j, st:st + CH, :]
                ls.append(l)
            rs = [pltpu.roll(l, 64, 1) for l in ls]
            return gs, pq, ls, rs

        def stage2(st1):
            gs, pq, ls, rs = st1
            ls = [l + r for l, r in zip(ls, rs)]
            rs = [pltpu.roll(l, 32, 1) for l in ls]
            return gs, pq, ls, rs

        def stage3(a0, CH, st2):
            gs, pq, ls, rs = st2
            ls = [l + r for l, r in zip(ls, rs)]
            g = jax.nn.sigmoid(gs)
            fa = g * _rcp(ls[0] + 1e-6)
            ls = ls[1:]
            if a0 < HALO:
                row = a0 + lax.broadcasted_iota(jnp.int32, (CH, 128), 0)
                ls = [ls[0]] + [jnp.where(row >= DIL * w, ls[w], -1e9 * LOG2E) for w in range(1, W)]
            m = ls[0]
            for w in range(1, W):
                m = jnp.maximum(m, ls[w])
            es = [jnp.exp2(l - m) for l in ls]
            den = es[0]
            for w in range(1, W):
                den = den + es[w]
            fb = (1.0 - g) * _rcp(den)
            for j in range(4):
                acc = None
                for w in range(W):
                    st = HALO + a0 - DIL * w
                    term = es[w] * v_ref[j, st:st + CH, :]
                    acc = term if acc is None else acc + term
                lhs_ref[a0:a0 + CH, D + 128 * j:D + 128 * (j + 1)] = (acc * fb).astype(BF16)
                lhs_ref[a0:a0 + CH, 128 * j:128 * (j + 1)] = (pq[:, 128 * j:128 * (j + 1)] * fa).astype(BF16)

        a0 = r0
        for CH in pattern:
            stage3(a0, CH, stage2(stage1(a0, CH)))
            a0 += CH
        assert a0 == r0 + TS

    def outp(i, half):
        r0 = i * TS
        c0 = half * 256
        ob_ref[r0:r0 + TS, c0:c0 + 256] = _dot(lhs_ref[r0:r0 + TS, :], wout_ref[:, c0:c0 + 256]).astype(BF16)

    def perm_rows_store(slot, val, c):
        for hh in range(8):
            p0 = PS * (8 * c + hh)
            for j in range(val.shape[1] // 128):
                m_ref[slot + j, p0:p0 + DH, :] = val[DH * hh:DH * (hh + 1), 128 * j:128 * (j + 1)]

    def perm_rows_load(slot, row0):
        for d in range(DH):
            for j in range(4):
                wout_ref[row0 + d * 32:row0 + (d + 1) * 32, 128 * j:128 * (j + 1)] = (
                    m_ref[slot + j, pl.ds(d, 32, stride=PS), :].astype(BF16))

    for m in range(4):
        cp_w(m).wait()
    cp_wv.wait()
    cp_woa.wait()
    cp_wob.wait()
    cp_gw.wait()
    cp_x2(3).wait()
    p1_seg(6, 2)
    prep_w(0)
    for c in range(4):
        perm_rows_store(8, z_ref[128 * c:128 * (c + 1), :], c)
    zp = jnp.concatenate([m_ref[8, pl.ds(d, 32, stride=PS), :] for d in range(DH)], axis=0)
    zrow_ref[...] = jnp.broadcast_to(jnp.sum(zp.T, axis=0, keepdims=True), (8, D))
    r_i = lax.broadcasted_iota(jnp.int32, (128, 128), 0) // DH
    c_i = lax.broadcasted_iota(jnp.int32, (128, 128), 1) // DH
    bd = r_i == c_i
    kvs = []
    for c in range(4):
        gc = g_ref[128 * c:128 * (c + 1), :].astype(BF16)
        kvs.append(jnp.where(bd, _dot(gc, wv_ref[:, 128 * c:128 * (c + 1)]), 0.0).astype(BF16))
    for c in range(4):
        mc = _dot(kvs[c], woa_ref[128 * c:128 * (c + 1), :])
        perm_rows_store(0, mc, c)
    for p in range(4):
        if p > 0:
            prep_w(p)
        proj(0, p)
        proj(1, p)

    P = lambda i: [("P", i, p) for p in range(4)]
    O = lambda t: [("O", t, 0), ("O", t, 1)]
    sched = [
        P(2) + P(3) + P(4)[:1],
        P(4)[1:] + P(5) + O(0),
        P(6) + P(7) + O(1)[:1],
        O(1)[1:] + O(2) + O(3) + O(4) + O(5),
    ]

    def mk_pattern(nf):
        n8 = (TS - 16 * nf) // 8
        pattern = []
        for c in range(n8 + nf):
            if nf and (c * nf) // (n8 + nf) != ((c + 1) * nf) // (n8 + nf):
                pattern.append(16)
            else:
                pattern.append(8)
        return pattern

    pending = []
    for s in range(4):
        barrier()
        for t in pending:
            cp_o(t).start()
        pending = []
        if s == 0:
            perm_rows_load(0, 0)
            for c in range(4):
                perm_rows_store(4, wob_ref[128 * c:128 * (c + 1), :].astype(F32), c)
            perm_rows_load(4, D)
        for (kind, t, p) in sched[s]:
            if kind == "P":
                proj(t, p)
            else:
                outp(t, p)
                if p == 1:
                    if s == 3:
                        cp_o(t).start()
                    else:
                        pending.append(t)
        attn(2 * s, mk_pattern(NFS[s]))
        attn(2 * s + 1, mk_pattern(NFS[s]))
    barrier()
    outp(NT - 2, 0)
    outp(NT - 2, 1)
    cp_o(NT - 2).start()
    last = []
    r7 = (NT - 1) * TS
    for (c0, nc) in [(0, 256), (256, 128), (384, 128)]:
        ob_ref[r7:r7 + TS, c0:c0 + nc] = _dot(lhs_ref[r7:r7 + TS, :], wout_ref[:, c0:c0 + nc]).astype(BF16)
        c = pltpu.make_async_copy(ob_ref.at[pl.ds(r7, TS), pl.ds(c0, nc)],
                                  o_hbm.at[pl.ds(r7, TS), pl.ds(c0, nc)], sem_d.at[4])
        c.start()
        last.append(c)
    for t in range(NT - 1):
        cp_o(t).wait()
    for c in last:
        c.wait()


@jax.jit
def pallas_gated_mix__linear_attn_block__sliding_local_dilated__prompt_kernel(
    A_x, A_wqkv, A_wo, B_x, B_wqkv, B_wo, gate_w,
):
    del B_x
    x = A_x.reshape(S, D)
    any_spec = pl.BlockSpec(memory_space=pl.ANY)
    out = pl.pallas_call(
        _kernel,
        out_shape=jax.ShapeDtypeStruct((S, D), BF16),
        in_specs=[any_spec] * 6,
        out_specs=any_spec,
        scratch_shapes=[
            pltpu.VMEM((S, D), BF16),
            pltpu.VMEM((2, D, 256), BF16),
            pltpu.VMEM((4, D, D), BF16),
            pltpu.VMEM((D, D), BF16),
            pltpu.VMEM((D, D), BF16),
            pltpu.VMEM((D, D), BF16),
            pltpu.VMEM((D,), BF16),
            pltpu.VMEM((D, D), BF16),
            pltpu.VMEM((D, D), F32),
            pltpu.VMEM((D, 128), F32),
            pltpu.VMEM((8, 4, 16 * PS, 128), F32),
            pltpu.VMEM((4 * D, D), BF16),
            pltpu.VMEM((2 * D, D), BF16),
            pltpu.VMEM((9, 32 * PS, 128), F32),
            pltpu.VMEM((8, D), F32),
            pltpu.VMEM((4, HALO + S, 128), F32),
            pltpu.VMEM((4, HALO + S, 128), F32),
            pltpu.VMEM((S, 2 * D), F32),
            pltpu.VMEM((S, 2 * D), BF16),
            pltpu.VMEM((S, D), BF16),
            pltpu.SemaphoreType.DMA((5,)),
            pltpu.SemaphoreType.REGULAR,
        ],
        compiler_params=pltpu.CompilerParams(vmem_limit_bytes=100 * 1024 * 1024),
    )(x, A_wqkv, A_wo, B_wqkv, B_wo, gate_w)
    return out.reshape(1, S, D)
```

```python
import jax
import jax.numpy as jnp
from jax import lax
import jax.experimental.pallas as pl
import jax.experimental.pallas.tpu as pltpu

S, D, H, DH = 2048, 512, 32, 16
W, DIL = 8, 2
TS = 256
NT = S // TS
HALO = 16
PS = 17
F32 = jnp.float32
BF16 = jnp.bfloat16
LOG2E = 1.4426950408889634
NT_DIMS = (((1,), (1,)), ((), ()))


def _phi(t):
    return jnp.where(t > 0, t + 1.0, jnp.exp(t)) + 1e-6


def _dot(a, b):
    return jnp.dot(a, b, preferred_element_type=F32)


def _dot_nt(a, b):
    return lax.dot_general(a, b, NT_DIMS, preferred_element_type=F32)


def _rcp(x):
    r = pl.reciprocal(x, approx=True)
    return r * (2.0 - x * r)


def _kernel(x_hbm, wa_hbm, woa_hbm, wb_hbm, wob_hbm, gw_hbm, o_hbm,
            x_ref, wk_ref, wnat_ref, wv_ref, woa_ref, wob_ref, gw_ref,
            wkT_ref, g_ref, z_ref, tmp_ref, w2T_ref, wout_ref, m_ref, zrow_ref,
            k_ref, v_ref, q_ref, lhs_ref, ob_ref,
            sem_d, sem_b):
    def barrier():
        pl.semaphore_signal(sem_b, 1)
        pl.semaphore_wait(sem_b, 1)

    def cp_x1(i):
        return pltpu.make_async_copy(x_hbm.at[pl.ds(i * TS, TS), :], x_ref.at[pl.ds(i * TS, TS), :], sem_d.at[i])

    def cp_x2(p):
        r = p * 2 * TS
        return pltpu.make_async_copy(x_hbm.at[pl.ds(r, 2 * TS), :], x_ref.at[pl.ds(r, 2 * TS), :],
                                     sem_d.at[2 if p < 3 else 3])

    def cp_w(m):
        src = wa_hbm.at[:, pl.ds(0, D)] if m == 0 else wb_hbm.at[:, pl.ds((m - 1) * D, D)]
        return pltpu.make_async_copy(src, wnat_ref.at[m], sem_d.at[3])

    def cp_wk(hf):
        return pltpu.make_async_copy(wa_hbm.at[:, pl.ds(D + hf * 256, 256)], wk_ref.at[hf], sem_d.at[hf])

    cp_wv = pltpu.make_async_copy(wa_hbm.at[:, pl.ds(2 * D, D)], wv_ref, sem_d.at[3])
    cp_woa = pltpu.make_async_copy(woa_hbm, woa_ref, sem_d.at[3])
    cp_wob = pltpu.make_async_copy(wob_hbm, wob_ref, sem_d.at[3])
    cp_gw = pltpu.make_async_copy(gw_hbm, gw_ref, sem_d.at[3])

    def cp_o(i):
        return pltpu.make_async_copy(ob_ref.at[pl.ds(i * TS, TS), :], o_hbm.at[pl.ds(i * TS, TS), :], sem_d.at[4])

    def prep_w(m):
        for hf in range(2):
            wt = wnat_ref[m, :, hf * 256:(hf + 1) * 256].astype(F32).T
            for hh in range(16):
                for j in range(4):
                    tmp_ref[2 * m + hf, j, PS * hh:PS * hh + DH, :] = wt[DH * hh:DH * (hh + 1), 128 * j:128 * (j + 1)]
            base = m * D + hf * 16
            for d in range(DH):
                r = base + d * 32
                for j in range(4):
                    w2T_ref[pl.ds(r, 16), 128 * j:128 * (j + 1)] = (
                        tmp_ref[2 * m + hf, j, pl.ds(d, 16, stride=PS), :].astype(BF16))

    cp_x1(0).start()
    cp_wk(0).start()
    cp_wk(1).start()
    cp_x1(1).start()
    cp_x2(1).start()
    cp_x2(2).start()
    k_ref[:, 0:HALO, :] = jnp.zeros((4, HALO, 128), F32)
    v_ref[:, 0:HALO, :] = jnp.zeros((4, HALO, 128), F32)

    for hf in range(2):
        cp_x1(hf).wait()
        cp_wk(hf).wait()
        if hf == 0:
            cp_x2(3).start()
            cp_w(0).start()
            cp_w(1).start()
            cp_w(2).start()
        else:
            cp_w(3).start()
            cp_wv.start()
            cp_woa.start()
            cp_wob.start()
            cp_gw.start()
        x0 = x_ref[0:TS, :]
        pkT = _phi(_dot(x0, wk_ref[hf])).T
        zs = pkT[:, 0:128]
        for j in range(1, TS // 128):
            zs = zs + pkT[:, 128 * j:128 * (j + 1)]
        z_ref[hf * 256:(hf + 1) * 256, :] = zs
        g_ref[hf * 256:(hf + 1) * 256, :] = _dot(pkT.astype(BF16), x0)
        wkT_ref[hf * 256:(hf + 1) * 256, :] = wk_ref[hf].astype(F32).T.astype(BF16)

    def p1_seg(t0, nt):
        n = nt * TS
        r0 = t0 * TS
        xt = x_ref[pl.ds(r0, n), :]
        kT = _dot_nt(wkT_ref[...], xt)
        pk = _phi(kT)
        zs = pk[:, 0:128]
        for j in range(1, n // 128):
            zs = zs + pk[:, 128 * j:128 * (j + 1)]
        z_ref[...] += zs
        g_ref[...] += _dot(pk.astype(BF16), xt)

    p1_seg(1, 1)

    cp_x2(1).wait()
    cp_x2(2).wait()
    p1_seg(2, 2)
    p1_seg(4, 2)

    def proj(i, part):
        r0 = i * TS
        xt = x_ref[r0:r0 + TS, :]
        pr = _dot_nt(xt, w2T_ref[part * D:(part + 1) * D, :])
        if part == 0:
            q_ref[r0:r0 + TS, 0:D] = pr
        elif part == 1:
            q_ref[r0:r0 + TS, D:2 * D] = pr * (0.25 * LOG2E)
        else:
            dst = k_ref if part == 2 else v_ref
            for j in range(4):
                dst[j, HALO + r0:HALO + r0 + TS, :] = pr[:, 128 * j:128 * (j + 1)]

    N8 = 6
    GR = N8 * 8 + 16

    def attn_rows(row0, ngroups, peel_first):
        zrow = zrow_ref[0:1, :]
        gw = gw_ref[...].reshape(1, D).astype(F32)

        def stage1(a0, CH):
            gs = jnp.sum(x_ref[pl.ds(a0, CH), :].astype(F32) * gw, axis=1, keepdims=True)
            pq = _phi(q_ref[pl.ds(a0, CH), 0:D])
            t = pq * zrow
            t = t[:, 0:128] + t[:, 128:256] + t[:, 256:384] + t[:, 384:512]
            q = [q_ref[pl.ds(a0, CH), D + 128 * j:D + 128 * (j + 1)] for j in range(4)]
            ls = [t]
            for w in range(W):
                st = HALO + a0 - DIL * w
                l = q[0] * k_ref[0, pl.ds(st, CH), :]
                for j in range(1, 4):
                    l = l + q[j] * k_ref[j, pl.ds(st, CH), :]
                ls.append(l)
            rs = [pltpu.roll(l, 64, 1) for l in ls]
            return gs, pq, ls, rs

        def stage2(st1):
            gs, pq, ls, rs = st1
            ls = [l + r for l, r in zip(ls, rs)]
            rs = [pltpu.roll(l, 32, 1) for l in ls]
            return gs, pq, ls, rs

        def stage3(a0, CH, st2):
            gs, pq, ls, rs = st2
            ls = [l + r for l, r in zip(ls, rs)]
            g = jax.nn.sigmoid(gs)
            fa = g * _rcp(ls[0] + 1e-6)
            ls = ls[1:]
            if isinstance(a0, int) and a0 < HALO:
                row = a0 + lax.broadcasted_iota(jnp.int32, (CH, 128), 0)
                ls = [ls[0]] + [jnp.where(row >= DIL * w, ls[w], -1e9 * LOG2E) for w in range(1, W)]
            m = ls[0]
            for w in range(1, W):
                m = jnp.maximum(m, ls[w])
            es = [jnp.exp2(l - m) for l in ls]
            den = es[0]
            for w in range(1, W):
                den = den + es[w]
            fb = (1.0 - g) * _rcp(den)
            for j in range(4):
                acc = None
                for w in range(W):
                    st = HALO + a0 - DIL * w
                    term = es[w] * v_ref[j, pl.ds(st, CH), :]
                    acc = term if acc is None else acc + term
                lhs_ref[pl.ds(a0, CH), D + 128 * j:D + 128 * (j + 1)] = (acc * fb).astype(BF16)
                lhs_ref[pl.ds(a0, CH), 128 * j:128 * (j + 1)] = (pq[:, 128 * j:128 * (j + 1)] * fa).astype(BF16)

        def chunk(a0, CH):
            if not isinstance(a0, int):
                a0 = pl.multiple_of(a0, 8)
            stage3(a0, CH, stage2(stage1(a0, CH)))

        def group(base, c0):
            def body8(ci, carry):
                chunk(base + ci * 8, 8)
                return carry

            lax.fori_loop(c0, N8, body8, 0, unroll=True)
            chunk(base + N8 * 8, 16)

        g0 = 0
        if peel_first:
            chunk(row0, 8)
            chunk(row0 + 8, 8)
            group(row0, 2)
            g0 = 1

        def body(gi, carry):
            group(pl.multiple_of(row0 + gi * GR, GR), 0)
            return carry

        lax.fori_loop(g0, ngroups, body, 0, unroll=True)

    def outp(i, half):
        r0 = i * TS
        c0 = half * 256
        ob_ref[r0:r0 + TS, c0:c0 + 256] = _dot(lhs_ref[r0:r0 + TS, :], wout_ref[:, c0:c0 + 256]).astype(BF16)

    def perm_rows_store(slot, val, c):
        for hh in range(8):
            p0 = PS * (8 * c + hh)
            for j in range(val.shape[1] // 128):
                m_ref[slot + j, p0:p0 + DH, :] = val[DH * hh:DH * (hh + 1), 128 * j:128 * (j + 1)]

    def perm_rows_load(slot, row0):
        for d in range(DH):
            for j in range(4):
                wout_ref[row0 + d * 32:row0 + (d + 1) * 32, 128 * j:128 * (j + 1)] = (
                    m_ref[slot + j, pl.ds(d, 32, stride=PS), :].astype(BF16))

    for m in range(4):
        cp_w(m).wait()
    cp_wv.wait()
    cp_woa.wait()
    cp_wob.wait()
    cp_gw.wait()
    cp_x2(3).wait()
    p1_seg(6, 2)
    prep_w(0)
    for c in range(4):
        perm_rows_store(8, z_ref[128 * c:128 * (c + 1), :], c)
    zp = jnp.concatenate([m_ref[8, pl.ds(d, 32, stride=PS), :] for d in range(DH)], axis=0)
    zrow_ref[...] = jnp.broadcast_to(jnp.sum(zp.T, axis=0, keepdims=True), (8, D))
    r_i = lax.broadcasted_iota(jnp.int32, (128, 128), 0) // DH
    c_i = lax.broadcasted_iota(jnp.int32, (128, 128), 1) // DH
    bd = r_i == c_i
    kvs = []
    for c in range(4):
        gc = g_ref[128 * c:128 * (c + 1), :].astype(BF16)
        kvs.append(jnp.where(bd, _dot(gc, wv_ref[:, 128 * c:128 * (c + 1)]), 0.0).astype(BF16))
    for c in range(4):
        mc = _dot(kvs[c], woa_ref[128 * c:128 * (c + 1), :])
        perm_rows_store(0, mc, c)
    for p in range(4):
        if p > 0:
            prep_w(p)
        proj(0, p)
        proj(1, p)

    P = lambda i: [("P", i, p) for p in range(4)]
    O = lambda t: [("O", t, 0), ("O", t, 1)]
    sched = [
        P(2) + P(3) + P(4)[:1],
        P(4)[1:] + P(5) + O(0),
        P(6) + P(7) + O(1)[:1],
        O(1)[1:] + O(2) + O(3) + O(4) + O(5),
    ]

    pending = []
    for s in range(4):
        barrier()
        for t in pending:
            cp_o(t).start()
        pending = []
        if s == 0:
            perm_rows_load(0, 0)
            for c in range(4):
                perm_rows_store(4, wob_ref[128 * c:128 * (c + 1), :].astype(F32), c)
            perm_rows_load(4, D)
        for (kind, t, p) in sched[s]:
            if kind == "P":
                proj(t, p)
            else:
                outp(t, p)
                if p == 1:
                    if s == 3:
                        cp_o(t).start()
                    else:
                        pending.append(t)
        attn_rows(2 * s * TS, 2 * TS // GR, s == 0)
    barrier()
    outp(NT - 2, 0)
    outp(NT - 2, 1)
    cp_o(NT - 2).start()
    last = []
    r7 = (NT - 1) * TS
    for (c0, nc) in [(0, 256), (256, 128), (384, 128)]:
        ob_ref[r7:r7 + TS, c0:c0 + nc] = _dot(lhs_ref[r7:r7 + TS, :], wout_ref[:, c0:c0 + nc]).astype(BF16)
        c = pltpu.make_async_copy(ob_ref.at[pl.ds(r7, TS), pl.ds(c0, nc)],
                                  o_hbm.at[pl.ds(r7, TS), pl.ds(c0, nc)], sem_d.at[4])
        c.start()
        last.append(c)
    for t in range(NT - 1):
        cp_o(t).wait()
    for c in last:
        c.wait()


@jax.jit
def pallas_gated_mix__linear_attn_block__sliding_local_dilated__prompt_kernel(
    A_x, A_wqkv, A_wo, B_x, B_wqkv, B_wo, gate_w,
):
    del B_x
    x = A_x.reshape(S, D)
    any_spec = pl.BlockSpec(memory_space=pl.ANY)
    out = pl.pallas_call(
        _kernel,
        out_shape=jax.ShapeDtypeStruct((S, D), BF16),
        in_specs=[any_spec] * 6,
        out_specs=any_spec,
        scratch_shapes=[
            pltpu.VMEM((S, D), BF16),
            pltpu.VMEM((2, D, 256), BF16),
            pltpu.VMEM((4, D, D), BF16),
            pltpu.VMEM((D, D), BF16),
            pltpu.VMEM((D, D), BF16),
            pltpu.VMEM((D, D), BF16),
            pltpu.VMEM((D,), BF16),
            pltpu.VMEM((D, D), BF16),
            pltpu.VMEM((D, D), F32),
            pltpu.VMEM((D, 128), F32),
            pltpu.VMEM((8, 4, 16 * PS, 128), F32),
            pltpu.VMEM((4 * D, D), BF16),
            pltpu.VMEM((2 * D, D), BF16),
            pltpu.VMEM((9, 32 * PS, 128), F32),
            pltpu.VMEM((8, D), F32),
            pltpu.VMEM((4, HALO + S, 128), F32),
            pltpu.VMEM((4, HALO + S, 128), F32),
            pltpu.VMEM((S, 2 * D), F32),
            pltpu.VMEM((S, 2 * D), BF16),
            pltpu.VMEM((S, D), BF16),
            pltpu.SemaphoreType.DMA((5,)),
            pltpu.SemaphoreType.REGULAR,
        ],
        compiler_params=pltpu.CompilerParams(vmem_limit_bytes=100 * 1024 * 1024),
    )(x, A_wqkv, A_wo, B_wqkv, B_wo, gate_w)
    return out.reshape(1, S, D)
```
